```python
import os as _os
_os.environ.setdefault("JAX_PLATFORMS", "cpu")
import jax
import jax.numpy as jnp

def _softmax(x, axis=-1):
    return jax.nn.softmax(x, axis=axis)
def _gelu(x):
    return jax.nn.gelu(x, approximate=True)
def _silu(x):
    return jax.nn.silu(x)
def _sigmoid(x):
    return jax.nn.sigmoid(x)
def _layernorm(x, axis=-1, eps=1e-5):
    m = jnp.mean(x, axis=axis, keepdims=True)
    v = jnp.var(x, axis=axis, keepdims=True)
    return (x - m) / jnp.sqrt(v + eps)
def _scatter_add(tgt, idx, src, axis=0):
    return tgt.at[idx].add(src)
def _segment_sum(src, seg, n):
    return jax.ops.segment_sum(src, seg, n)
class _Rng:
    def __init__(self, key):
        self._k = key
    def _next(self):
        self._k, sub = jax.random.split(self._k)
        return sub
    def normal(self, shape):
        return jax.random.normal(self._next(), shape, dtype=jnp.bfloat16)
    def randint(self, lo, hi, shape):
        return jax.random.randint(self._next(), shape, lo, hi, dtype=jnp.int32)
    def uniform(self, shape, lo=0.0, hi=1.0):
        return jax.random.uniform(self._next(), shape, jnp.bfloat16, lo, hi)
    def permutation(self, n):
        return jax.random.permutation(self._next(), n)


kernel_name = 'concat_heads__grouped_kv_mqa__sliding_block__prompt'

def setup_inputs():
    _rng = _Rng(jax.random.key(int.from_bytes(__import__("os").urandom(4), "little")))
    _w = (lambda a: (lambda t: t.astype(jnp.bfloat16) if jnp.issubdtype(t.dtype, jnp.floating) else t)(jnp.asarray(a)))
    def _A_setup():
        B, S, D, H = 1, 2048, 1024, 32
        Dh = D // H
        return {
            "x": _w((lambda *s: _rng.normal(s) * 0.05)(B, S, D)),
            "wq": _w((lambda *s: _rng.normal(s) * 1.6)(D, H * Dh)),
            "wk": _w((lambda *s: _rng.normal(s) * 1.6)(D, Dh)),
            "wv": _w((lambda *s: _rng.normal(s) * 0.1)(D, Dh)),
            "wo": _w((lambda *s: _rng.normal(s) * 0.1)(H * Dh, D)),
        }
    _A_in = _A_setup()

    def _B_setup():
        B, S, D = 1, 2048, 1024
        return {
            "x": _w((lambda *s: _rng.normal(s) * 0.2)(B, S, D)),
            "wqkv": _w((lambda *s: _rng.normal(s) * 0.2)(D, 3 * D)),
            "wo": _w((lambda *s: _rng.normal(s) * 0.05)(D, D)),
        }
    _B_in = _B_setup()

    return {
        "A_x": _A_in["x"],
        "A_wq": _A_in["wq"],
        "A_wk": _A_in["wk"],
        "A_wv": _A_in["wv"],
        "A_wo": _A_in["wo"],
        "B_x": _B_in["x"],
        "B_wqkv": _B_in["wqkv"],
        "B_wo": _B_in["wo"],
    }

def reference(A_x, A_wq, A_wk, A_wv, A_wo, B_x, B_wqkv, B_wo):
    def _A_ref(x, wq, wk, wv, wo):
        B, S, D = x.shape
        H = 32
        Dh = D // H
        q = (lambda x, *d: x.transpose(*d))((x @ wq).reshape(B, S, H, Dh), 0, 2, 1, 3)
        k = x @ wk
        v = x @ wv
        scores = jnp.einsum("bhqd,bkd->bhqk", q, k) * (Dh ** -0.5)
        p = _softmax(scores, axis=-1)
        o = jnp.einsum("bhqk,bkd->bhqd", p, v)
        return (lambda x, *d: x.transpose(*d))(o, 0, 2, 1, 3).reshape(B, S, H * Dh) @ wo

    def _B_ref(x, wqkv, wo):
        B, S, D = x.shape
        H = 32; Dh = D // H; W = 256
        qkv = (lambda x, *d: x.transpose(*d))((x @ wqkv).reshape(B, S, 3, H, Dh), 2, 0, 3, 1, 4)
        q, k, v = qkv[0], qkv[1], qkv[2]
        scores = jnp.einsum("bhqd,bhkd->bhqk", q, k) * (Dh ** -0.5)
        idx = jnp.arange(S)
        mask = (idx[:, None] - idx[None, :] >= 0) & (idx[:, None] - idx[None, :] < W)
        scores = jnp.where(mask[None, None], scores, -1e9)
        p = _softmax(scores, axis=-1)
        o = jnp.einsum("bhqk,bhkd->bhqd", p, v)
        return (lambda x, *d: x.transpose(*d))(o, 0, 2, 1, 3).reshape(B, S, D) @ wo

    a = _A_ref(A_x, A_wq, A_wk, A_wv, A_wo)
    b = _B_ref(B_x, B_wqkv, B_wo)
    return jnp.concatenate([a, b], axis=-1)
```

```python
import functools
import jax
import jax.numpy as jnp
from jax import lax
from jax.experimental import pallas as pl
from jax.experimental.pallas import tpu as pltpu

S = 2048
D = 1024
H = 32
DH = 32
W = 256
KW = W + 128
LOG2E = 1.4426950408889634
QSCALE = (DH ** -0.5) * LOG2E
NEG = -1e30
NT = (((1,), (1,)), ((), ()))
TN = (((0,), (0,)), ((), ()))


def _kernel(ax_hbm, awq_hbm, awkt_hbm, awvt_hbm, awo_hbm, bx_hbm, bwqkv_hbm, bwo_hbm,
            o_hbm,
            ax_ref, awq_ref, wkv_ref, awo_ref, bx_ref, bwqkv_ref, bwo_ref, oa_ref, ob_ref,
            in_sems, out_sems,
            ka_ref, vta_ref, kb_ref, vtb_ref, qt_ref, ot_ref, s_ref, m_ref,
            sb_ref, mb_ref, bias_ref, *, tq):
    i = pl.program_id(0)
    nb = pl.num_programs(0)
    f32 = jnp.float32
    bf16 = jnp.bfloat16
    nr = tq // 128
    nch = S // tq

    def ax_copy(c):
        return pltpu.make_async_copy(ax_hbm.at[pl.ds(c * tq, tq)], ax_ref.at[pl.ds(c * tq, tq)], in_sems.at[c])
    wq_copy = pltpu.make_async_copy(awq_hbm, awq_ref, in_sems.at[nch])
    wk_copy = pltpu.make_async_copy(awkt_hbm, wkv_ref.at[pl.ds(0, DH)], in_sems.at[nch + 1])
    wv_copy = pltpu.make_async_copy(awvt_hbm, wkv_ref.at[pl.ds(DH, DH)], in_sems.at[nch + 2])
    wo_copy = pltpu.make_async_copy(awo_hbm, awo_ref, in_sems.at[nch + 3])
    bx_copy = pltpu.make_async_copy(bx_hbm, bx_ref, in_sems.at[nch + 4])
    wqkv_copy = pltpu.make_async_copy(bwqkv_hbm, bwqkv_ref, in_sems.at[nch + 5])
    bwo_copy = pltpu.make_async_copy(bwo_hbm, bwo_ref, in_sems.at[nch + 6])

    q0 = pl.multiple_of(i * tq, tq)

    def out_copy(step, half):
        r0 = pl.multiple_of(step * tq, tq)
        src = oa_ref if half == 0 else ob_ref
        return pltpu.make_async_copy(src, o_hbm.at[pl.ds(r0, tq), pl.ds(half * D, D)], out_sems.at[half])

    @pl.when(i == 0)
    def _start():
        ax_copy(0).start()
        wq_copy.start()
        wk_copy.start()
        wv_copy.start()
        for c in range(1, nch):
            ax_copy(c).start()
        wo_copy.start()
        bx_copy.start()
        wqkv_copy.start()
        bwo_copy.start()
        kb_ref[pl.ds(0, W), :] = jnp.zeros((W, D), bf16)
        vtb_ref[:, pl.ds(0, W)] = jnp.zeros((D, W), bf16)
        ax_copy(0).wait()
        wq_copy.wait()

    xa = ax_ref[pl.ds(q0, tq), :]
    qa = jnp.dot(xa, awq_ref[...], preferred_element_type=f32) * QSCALE
    qt_ref[...] = qa.T.astype(bf16)

    @pl.when(i == 0)
    def _kv():
        wk_copy.wait()
        wv_copy.wait()
        for c in range(nch):
            if c > 0:
                ax_copy(c).wait()
            kvt = lax.dot_general(wkv_ref[...], ax_ref[pl.ds(c * tq, tq), :], NT,
                                  preferred_element_type=f32)
            ka_ref[pl.ds(c * tq, tq), :] = kvt[0:DH, :].T.astype(bf16)
            vta_ref[:, pl.ds(c * tq, tq)] = kvt[DH:2 * DH, :].astype(bf16)

    def a_qk(h, slot):
        r0 = pl.multiple_of(h * DH, DH)
        qth = qt_ref[pl.ds(r0, DH), :]
        st = jnp.dot(ka_ref[...], qth, preferred_element_type=f32)
        s_ref[slot] = st
        m_ref[slot] = jnp.max(st, axis=0, keepdims=True)

    def a_pv(h, slot):
        r0 = pl.multiple_of(h * DH, DH)
        p = jnp.exp2(s_ref[slot] - m_ref[slot])
        l = jnp.sum(p, axis=0, keepdims=True)
        ot = jnp.dot(vta_ref[...], p.astype(bf16), preferred_element_type=f32)
        ot_ref[pl.ds(r0, DH), :] = (ot / l).astype(bf16)

    a_qk(0, 0)

    def a_body(j, carry):
        h = 2 * j
        a_qk(h + 1, 1)
        a_pv(h, 0)
        a_qk(h + 2, 0)
        a_pv(h + 1, 1)
        return carry

    lax.fori_loop(0, H // 2 - 1, a_body, 0)
    a_qk(H - 1, 1)
    a_pv(H - 2, 0)
    a_pv(H - 1, 1)

    @pl.when(i == 0)
    def _w1():
        wo_copy.wait()
        bx_copy.wait()
        wqkv_copy.wait()
        bwo_copy.wait()

    @pl.when(i > 0)
    def _w2():
        out_copy(i - 1, 0).wait()

    outa = lax.dot_general(ot_ref[...], awo_ref[...], TN, preferred_element_type=f32)
    oa_ref[...] = outa.astype(bf16)
    out_copy(i, 0).start()

    xb = bx_ref[pl.ds(q0, tq), :]
    qb = jnp.dot(xb, bwqkv_ref[:, pl.ds(0, D)], preferred_element_type=f32) * QSCALE
    qt_ref[...] = qb.T.astype(bf16)
    kb = jnp.dot(xb, bwqkv_ref[:, pl.ds(D, D)], preferred_element_type=f32)
    kb_ref[pl.ds(W + q0, tq), :] = kb.astype(bf16)
    vb = jnp.dot(xb, bwqkv_ref[:, pl.ds(2 * D, D)], preferred_element_type=f32)
    vtb_ref[:, pl.ds(W + q0, tq)] = vb.T.astype(bf16)

    ri = lax.broadcasted_iota(jnp.int32, (KW, 128), 0)
    cj = lax.broadcasted_iota(jnp.int32, (KW, 128), 1)
    band = (ri > cj) & (ri <= cj + W)
    for r in range(nr):
        qs = q0 + r * 128
        valid = band & (ri >= W - qs)
        bias_ref[r] = jnp.where(valid, 0.0, NEG).astype(f32)

    rsel = lax.broadcasted_iota(jnp.int32, (128, 512), 0) // DH
    csel = lax.broadcasted_iota(jnp.int32, (128, 512), 1) // 128
    diag = rsel == csel

    def b_qk(n, slot):
        r = n // 8
        g = n % 8
        g0 = pl.multiple_of(g * 128, 128)
        c0 = pl.multiple_of(r * 128, 128)
        ks = pl.multiple_of(q0 + r * 128, 128)
        q4 = qt_ref[pl.ds(g0, 128), pl.ds(c0, 128)]
        q4r = jnp.concatenate([q4, q4, q4, q4], axis=1)
        rhs = jnp.where(diag, q4r, jnp.zeros_like(q4r))
        k4 = kb_ref[pl.ds(ks, KW), pl.ds(g0, 128)]
        st = jnp.dot(k4, rhs, preferred_element_type=f32)
        b = bias_ref[r]
        st = st + jnp.concatenate([b, b, b, b], axis=1)
        sb_ref[slot] = st
        mb_ref[slot] = jnp.max(st, axis=0, keepdims=True)

    def b_pv(n, slot):
        r = n // 8
        g = n % 8
        c0 = pl.multiple_of(r * 128, 128)
        ks = pl.multiple_of(q0 + r * 128, 128)
        for j in range(4):
            p = jnp.exp2(sb_ref[slot, :, pl.ds(j * 128, 128)] - mb_ref[slot, :, pl.ds(j * 128, 128)])
            l = jnp.sum(p, axis=0, keepdims=True)
            rr = pl.multiple_of(g * 128 + j * DH, DH)
            vt = vtb_ref[pl.ds(rr, DH), pl.ds(ks, KW)]
            o = jnp.dot(vt, p.astype(bf16), preferred_element_type=f32)
            ot_ref[pl.ds(rr, DH), pl.ds(c0, 128)] = (o / l).astype(bf16)

    nitems = nr * 8
    b_qk(0, 0)

    def b_body(j, carry):
        n = 2 * j
        b_qk(n + 1, 1)
        b_pv(n, 0)
        b_qk(n + 2, 0)
        b_pv(n + 1, 1)
        return carry

    lax.fori_loop(0, nitems // 2 - 1, b_body, 0)
    b_qk(nitems - 1, 1)
    b_pv(nitems - 2, 0)
    b_pv(nitems - 1, 1)

    @pl.when(i > 0)
    def _w3():
        out_copy(i - 1, 1).wait()

    outb = lax.dot_general(ot_ref[...], bwo_ref[...], TN, preferred_element_type=f32)
    ob_ref[...] = outb.astype(bf16)
    out_copy(i, 1).start()

    @pl.when(i == nb - 1)
    def _fin():
        out_copy(i, 0).wait()
        out_copy(i, 1).wait()


TQ = 512
VMEM_MB = 80


@jax.jit
def pallas_concat_heads__grouped_kv_mqa__sliding_block__prompt_kernel(
        A_x, A_wq, A_wk, A_wv, A_wo, B_x, B_wqkv, B_wo):
    tq = TQ
    vmem_mb = VMEM_MB
    nb = S // tq
    bf16 = jnp.bfloat16
    f32 = jnp.float32
    anyspec = pl.BlockSpec(memory_space=pl.ANY)
    out = pl.pallas_call(
        functools.partial(_kernel, tq=tq),
        grid=(nb,),
        in_specs=[anyspec] * 8,
        out_specs=anyspec,
        out_shape=jax.ShapeDtypeStruct((S, 2 * D), bf16),
        scratch_shapes=[
            pltpu.VMEM((S, D), bf16),
            pltpu.VMEM((D, D), bf16),
            pltpu.VMEM((2 * DH, D), bf16),
            pltpu.VMEM((D, D), bf16),
            pltpu.VMEM((S, D), bf16),
            pltpu.VMEM((D, 3 * D), bf16),
            pltpu.VMEM((D, D), bf16),
            pltpu.VMEM((tq, D), bf16),
            pltpu.VMEM((tq, D), bf16),
            pltpu.SemaphoreType.DMA((S // tq + 7,)),
            pltpu.SemaphoreType.DMA((2,)),
            pltpu.VMEM((S, DH), bf16),
            pltpu.VMEM((DH, S), bf16),
            pltpu.VMEM((W + S, D), bf16),
            pltpu.VMEM((D, W + S), bf16),
            pltpu.VMEM((D, tq), bf16),
            pltpu.VMEM((D, tq), bf16),
            pltpu.VMEM((2, S, tq), f32),
            pltpu.VMEM((2, 1, tq), f32),
            pltpu.VMEM((2, KW, 512), f32),
            pltpu.VMEM((2, 1, 512), f32),
            pltpu.VMEM((tq // 128, KW, 128), f32),
        ],
        compiler_params=pltpu.CompilerParams(
            dimension_semantics=("arbitrary",),
            vmem_limit_bytes=vmem_mb * 1024 * 1024),
    )(A_x[0], A_wq, A_wk.T, A_wv.T, A_wo, B_x[0], B_wqkv, B_wo)
    return out[None]
```

```python
import functools
import jax
import jax.numpy as jnp
from jax import lax
from jax.experimental import pallas as pl
from jax.experimental.pallas import tpu as pltpu

S = 2048
D = 1024
H = 32
DH = 32
W = 256
KW = W + 128
LOG2E = 1.4426950408889634
QSCALE = (DH ** -0.5) * LOG2E
NEG = -1e30
NT = (((1,), (1,)), ((), ()))
TN = (((0,), (0,)), ((), ()))


def _kernel(ax_hbm, awq_hbm, awkt_hbm, awvt_hbm, awo_hbm, bx_hbm, bwqkv_hbm, bwo_hbm,
            o_hbm,
            ax_ref, awq_ref, wkv_ref, awo_ref, bx_ref, bwqkv_ref, bwo_ref, oa_ref, ob_ref,
            in_sems, out_sems,
            ka_ref, vta_ref, kb_ref, vtb_ref, qta_ref, ota_ref, qtb_ref, otb_ref,
            s0_ref, s1_ref, m_ref,
            sb0_ref, sb1_ref, mb_ref, bias_ref, *, tq, nc, gps):
    i = pl.program_id(0)
    nb = pl.num_programs(0)
    f32 = jnp.float32
    bf16 = jnp.bfloat16
    nr = tq // 128
    nch = S // tq

    def ax_copy(c):
        return pltpu.make_async_copy(ax_hbm.at[pl.ds(c * tq, tq)], ax_ref.at[pl.ds(c * tq, tq)], in_sems.at[c])
    wq_copy = pltpu.make_async_copy(awq_hbm, awq_ref, in_sems.at[nch])
    wk_copy = pltpu.make_async_copy(awkt_hbm, wkv_ref.at[pl.ds(0, DH)], in_sems.at[nch + 1])
    wv_copy = pltpu.make_async_copy(awvt_hbm, wkv_ref.at[pl.ds(DH, DH)], in_sems.at[nch + 2])
    wo_copy = pltpu.make_async_copy(awo_hbm, awo_ref, in_sems.at[nch + 3])
    bx_copy = pltpu.make_async_copy(bx_hbm, bx_ref, in_sems.at[nch + 4])
    wqkv_copy = pltpu.make_async_copy(bwqkv_hbm, bwqkv_ref, in_sems.at[nch + 5])
    bwo_copy = pltpu.make_async_copy(bwo_hbm, bwo_ref, in_sems.at[nch + 6])

    q0 = pl.multiple_of(i * tq, tq)

    def out_copy(step, half):
        r0 = pl.multiple_of(step * tq, tq)
        src = oa_ref if half == 0 else ob_ref
        return pltpu.make_async_copy(src, o_hbm.at[pl.ds(r0, tq), pl.ds(half * D, D)], out_sems.at[half])

    def qproj_a(step):
        r0 = pl.multiple_of(step * tq, tq)
        xa = ax_ref[pl.ds(r0, tq), :]
        qa = jnp.dot(xa, awq_ref[...], preferred_element_type=f32) * QSCALE
        qta_ref[...] = qa.T.astype(bf16)

    ck = S // nc
    s_refs = (s0_ref, s1_ref)

    def a_stage(hq, sq, hp, sp):
        if hq is not None:
            qth = qta_ref[pl.ds(pl.multiple_of(hq * DH, DH), DH), :]
            mq = None
        if hp is not None:
            mp = m_ref[sp]
            l8 = None
            acc = None
        for c in range(nc):
            rows = pl.ds(c * ck, ck)
            if hq is not None:
                st = jnp.dot(ka_ref[rows, :], qth, preferred_element_type=f32)
                s_refs[sq][rows, :] = st
                mc = jnp.max(st.reshape(ck // 8, 8, tq), axis=0)
                mq = mc if mq is None else jnp.maximum(mq, mc)
            if hp is not None:
                p = jnp.exp2(s_refs[sp][rows, :] - mp)
                lc = jnp.sum(p.reshape(ck // 8, 8, tq), axis=0)
                l8 = lc if l8 is None else l8 + lc
                oc = jnp.dot(vta_ref[:, rows], p.astype(bf16), preferred_element_type=f32)
                acc = oc if acc is None else acc + oc
        if hq is not None:
            m_ref[sq] = jnp.max(mq, axis=0, keepdims=True)
        if hp is not None:
            l = jnp.sum(l8, axis=0, keepdims=True)
            ota_ref[pl.ds(pl.multiple_of(hp * DH, DH), DH), :] = (acc / l).astype(bf16)

    @pl.when(i == 0)
    def _start():
        ax_copy(0).start()
        wq_copy.start()
        wk_copy.start()
        wv_copy.start()
        kb_ref[pl.ds(0, W), :] = jnp.zeros((W, D), bf16)
        vtb_ref[:, pl.ds(0, W)] = jnp.zeros((D, W), bf16)
        ax_copy(0).wait()
        wq_copy.wait()
        for c in range(1, nch):
            ax_copy(c).start()

    qproj_a(i)

    @pl.when(i == 0)
    def _kv():
        wk_copy.wait()
        wv_copy.wait()
        for c in range(nch):
            if c > 0:
                ax_copy(c).wait()
            if c == nch - 1:
                wo_copy.start()
                bx_copy.start()
                wqkv_copy.start()
                bwo_copy.start()
            kvt = lax.dot_general(wkv_ref[...], ax_ref[pl.ds(c * tq, tq), :], NT,
                                  preferred_element_type=f32)
            ka_ref[pl.ds(c * tq, tq), :] = kvt[0:DH, :].T.astype(bf16)
            vta_ref[:, pl.ds(c * tq, tq)] = kvt[DH:2 * DH, :].astype(bf16)

    a_stage(0, 0, None, None)

    def a_body(h, carry):
        par = h % 2

        @pl.when(par == 0)
        def _():
            a_stage(h + 1, 1, h, 0)

        @pl.when(par == 1)
        def _():
            a_stage(h + 1, 0, h, 1)
        return carry

    lax.fori_loop(0, H - 1, a_body, 0)

    @pl.when(i == 0)
    def _w1():
        wo_copy.wait()
        bx_copy.wait()
        wqkv_copy.wait()
        bwo_copy.wait()

    @pl.when(i > 0)
    def _w2():
        out_copy(i - 1, 0).wait()
        out_copy(i - 1, 1).wait()

    a_stage(None, None, H - 1, 1)

    xb = bx_ref[pl.ds(q0, tq), :]
    qb = jnp.dot(xb, bwqkv_ref[:, pl.ds(0, D)], preferred_element_type=f32) * QSCALE
    qtb_ref[...] = qb.T.astype(bf16)
    kb = jnp.dot(xb, bwqkv_ref[:, pl.ds(D, D)], preferred_element_type=f32)
    kb_ref[pl.ds(W + q0, tq), :] = kb.astype(bf16)
    vb = jnp.dot(xb, bwqkv_ref[:, pl.ds(2 * D, D)], preferred_element_type=f32)
    vtb_ref[:, pl.ds(W + q0, tq)] = vb.T.astype(bf16)

    ri = lax.broadcasted_iota(jnp.int32, (KW, 128), 0)
    cj = lax.broadcasted_iota(jnp.int32, (KW, 128), 1)
    band = (ri > cj) & (ri <= cj + W)
    for r in range(nr):
        qs = q0 + r * 128
        valid = band & (ri >= W - qs)
        bias_ref[r] = jnp.where(valid, 0.0, NEG).astype(f32)

    rsel = lax.broadcasted_iota(jnp.int32, (128, 128), 0) // DH
    sb_refs = (sb0_ref, sb1_ref)
    spr = 8 // gps

    def b_stage(nq, sq, np_, sp):
        if nq is not None:
            rq = nq // spr
            gq = (nq % spr) * gps
            cq = pl.multiple_of(rq * 128, 128)
            kq = pl.multiple_of(q0 + rq * 128, 128)
            b = bias_ref[rq]
        if np_ is not None:
            rp = np_ // spr
            gp = (np_ % spr) * gps
            c0 = pl.multiple_of(rp * 128, 128)
            ks = pl.multiple_of(q0 + rp * 128, 128)
        for u in range(gps):
            if nq is not None:
                g0 = pl.multiple_of((gq + u) * 128, 128)
                q4 = qtb_ref[pl.ds(g0, 128), pl.ds(cq, 128)]
                k4 = kb_ref[pl.ds(kq, KW), pl.ds(g0, 128)]
            for j in range(4):
                cols = pl.ds((u * 4 + j) * 128, 128)
                if nq is not None:
                    rhs = jnp.where(rsel == j, q4, jnp.zeros_like(q4))
                    st = jnp.dot(k4, rhs, preferred_element_type=f32) + b
                    sb_refs[sq][:, cols] = st
                    mb_ref[sq, :, cols] = jnp.max(st, axis=0, keepdims=True)
                if np_ is not None:
                    p = jnp.exp2(sb_refs[sp][:, cols] - mb_ref[sp, :, cols])
                    l = jnp.sum(p, axis=0, keepdims=True)
                    rr = pl.multiple_of((gp + u) * 128 + j * DH, DH)
                    vt = vtb_ref[pl.ds(rr, DH), pl.ds(ks, KW)]
                    o = jnp.dot(vt, p.astype(bf16), preferred_element_type=f32)
                    otb_ref[pl.ds(rr, DH), pl.ds(c0, 128)] = (o / l).astype(bf16)

    nitems = nr * spr
    b_stage(0, 0, None, None)

    def b_body(n, carry):
        par = n % 2

        @pl.when(par == 0)
        def _():
            b_stage(n + 1, 1, n, 0)

        @pl.when(par == 1)
        def _():
            b_stage(n + 1, 0, n, 1)
        return carry

    lax.fori_loop(0, nitems - 1, b_body, 0)
    b_stage(None, None, nitems - 1, 1)

    outa = lax.dot_general(ota_ref[...], awo_ref[...], TN, preferred_element_type=f32)
    oa_ref[...] = outa.astype(bf16)
    out_copy(i, 0).start()
    outb = lax.dot_general(otb_ref[...], bwo_ref[...], TN, preferred_element_type=f32)
    ob_ref[...] = outb.astype(bf16)
    out_copy(i, 1).start()

    @pl.when(i == nb - 1)
    def _fin():
        out_copy(i, 0).wait()
        out_copy(i, 1).wait()


@jax.jit
def pallas_concat_heads__grouped_kv_mqa__sliding_block__prompt_kernel(
        A_x, A_wq, A_wk, A_wv, A_wo, B_x, B_wqkv, B_wo):
    tq = 512
    vmem_mb = 80
    nc = 16
    gps = 4
    nb = S // tq
    bf16 = jnp.bfloat16
    f32 = jnp.float32
    anyspec = pl.BlockSpec(memory_space=pl.ANY)
    out = pl.pallas_call(
        functools.partial(_kernel, tq=tq, nc=nc, gps=gps),
        grid=(nb,),
        in_specs=[anyspec] * 8,
        out_specs=anyspec,
        out_shape=jax.ShapeDtypeStruct((S, 2 * D), bf16),
        scratch_shapes=[
            pltpu.VMEM((S, D), bf16),
            pltpu.VMEM((D, D), bf16),
            pltpu.VMEM((2 * DH, D), bf16),
            pltpu.VMEM((D, D), bf16),
            pltpu.VMEM((S, D), bf16),
            pltpu.VMEM((D, 3 * D), bf16),
            pltpu.VMEM((D, D), bf16),
            pltpu.VMEM((tq, D), bf16),
            pltpu.VMEM((tq, D), bf16),
            pltpu.SemaphoreType.DMA((S // tq + 7,)),
            pltpu.SemaphoreType.DMA((2,)),
            pltpu.VMEM((S, DH), bf16),
            pltpu.VMEM((DH, S), bf16),
            pltpu.VMEM((W + S, D), bf16),
            pltpu.VMEM((D, W + S), bf16),
            pltpu.VMEM((D, tq), bf16),
            pltpu.VMEM((D, tq), bf16),
            pltpu.VMEM((D, tq), bf16),
            pltpu.VMEM((D, tq), bf16),
            pltpu.VMEM((S, tq), f32),
            pltpu.VMEM((S, tq), f32),
            pltpu.VMEM((2, 1, tq), f32),
            pltpu.VMEM((KW, 512 * gps), f32),
            pltpu.VMEM((KW, 512 * gps), f32),
            pltpu.VMEM((2, 1, 512 * gps), f32),
            pltpu.VMEM((tq // 128, KW, 128), f32),
        ],
        compiler_params=pltpu.CompilerParams(
            dimension_semantics=("arbitrary",),
            vmem_limit_bytes=vmem_mb * 1024 * 1024),
    )(A_x[0], A_wq, A_wk.T, A_wv.T, A_wo, B_x[0], B_wqkv, B_wo)
    return out[None]
```
